```python
import os as _os
_os.environ.setdefault("JAX_PLATFORMS", "cpu")
import jax
import jax.numpy as jnp

def _softmax(x, axis=-1):
    return jax.nn.softmax(x, axis=axis)
def _gelu(x):
    return jax.nn.gelu(x, approximate=True)
def _silu(x):
    return jax.nn.silu(x)
def _sigmoid(x):
    return jax.nn.sigmoid(x)
def _layernorm(x, axis=-1, eps=1e-5):
    m = jnp.mean(x, axis=axis, keepdims=True)
    v = jnp.var(x, axis=axis, keepdims=True)
    return (x - m) / jnp.sqrt(v + eps)
def _scatter_add(tgt, idx, src, axis=0):
    return tgt.at[idx].add(src)
def _segment_sum(src, seg, n):
    return jax.ops.segment_sum(src, seg, n)
class _Rng:
    def __init__(self, key):
        self._k = key
    def _next(self):
        self._k, sub = jax.random.split(self._k)
        return sub
    def normal(self, shape):
        return jax.random.normal(self._next(), shape, dtype=jnp.bfloat16)
    def randint(self, lo, hi, shape):
        return jax.random.randint(self._next(), shape, lo, hi, dtype=jnp.int32)
    def uniform(self, shape, lo=0.0, hi=1.0):
        return jax.random.uniform(self._next(), shape, jnp.bfloat16, lo, hi)
    def permutation(self, n):
        return jax.random.permutation(self._next(), n)


kernel_name = 'interleave_layers__sliding_block__dense_activation_gelu__prompt'

def setup_inputs():
    _rng = _Rng(jax.random.key(int.from_bytes(__import__("os").urandom(4), "little")))
    _w = (lambda a: (lambda t: t.astype(jnp.bfloat16) if jnp.issubdtype(t.dtype, jnp.floating) else t)(jnp.asarray(a)))
    def _A_setup():
        B, S, D = 1, 2048, 640
        return {
            "x": _w((lambda *s: _rng.normal(s) * 0.05)(B, S, D)),
            "wqkv": _w((lambda *s: _rng.normal(s) * 0.05)(D, 3 * D)),
            "wo": _w((lambda *s: _rng.normal(s) * 0.05)(D, D)),
        }
    _A_in = _A_setup()

    def _B_setup():
        B, S, D, F = 1, 2048, 640, 1728
        return {
            "x": _w((lambda *s: _rng.normal(s) * 0.05)(B, S, D)),
            "w1": _w((lambda *s: _rng.normal(s) * 0.8)(D, F) * (D ** -0.5)),
            "b1": _w((lambda *s: _rng.normal(s) * 0.8)(F) * 0.01),
            "w2": _w((lambda *s: _rng.normal(s) * 0.8)(F, D) * (F ** -0.5)),
            "b2": _w((lambda *s: _rng.normal(s) * 0.8)(D) * 0.01),
        }
    _B_in = _B_setup()

    return {
        "A_x": _A_in["x"],
        "A_wqkv": _A_in["wqkv"],
        "A_wo": _A_in["wo"],
        "B_x": _B_in["x"],
        "B_w1": _B_in["w1"],
        "B_b1": _B_in["b1"],
        "B_w2": _B_in["w2"],
        "B_b2": _B_in["b2"],
    }

def reference(A_x, A_wqkv, A_wo, B_x, B_w1, B_b1, B_w2, B_b2):
    def _A_ref(x, wqkv, wo):
        B, S, D = x.shape
        H = 32; Dh = D // H; W = 256
        qkv = (lambda x, *d: x.transpose(*d))((x @ wqkv).reshape(B, S, 3, H, Dh), 2, 0, 3, 1, 4)
        q, k, v = qkv[0], qkv[1], qkv[2]
        scores = jnp.einsum("bhqd,bhkd->bhqk", q, k) * (Dh ** -0.5)
        idx = jnp.arange(S)
        mask = (idx[:, None] - idx[None, :] >= 0) & (idx[:, None] - idx[None, :] < W)
        scores = jnp.where(mask[None, None], scores, -1e9)
        p = _softmax(scores, axis=-1)
        o = jnp.einsum("bhqk,bhkd->bhqd", p, v)
        return (lambda x, *d: x.transpose(*d))(o, 0, 2, 1, 3).reshape(B, S, D) @ wo

    def _B_ref(x, w1, b1, w2, b2):
        h = jnp.einsum("bsd,df->bsf", x, w1) + b1
        h = _gelu(h)
        return jnp.einsum("bsf,fd->bsd", h, w2) + b2

    x = A_x
    x = x + _A_ref(_layernorm(x, axis=-1), A_wqkv, A_wo)
    x = x + _B_ref(_layernorm(x, axis=-1), B_w1, B_b1, B_w2, B_b2)
    x = x + _A_ref(_layernorm(x, axis=-1), A_wqkv, A_wo)
    x = x + _B_ref(_layernorm(x, axis=-1), B_w1, B_b1, B_w2, B_b2)
    return x
```

```python
import jax
import jax.numpy as jnp
from jax import lax
import jax.experimental.pallas as pl
import jax.experimental.pallas.tpu as pltpu

S, D, H, DH, W, F = 2048, 640, 32, 20, 256, 1728
BASES = (0, 120, 240, 360, 480, 512)
R = 256
UNR = 9
KC = 96
BF, F32 = jnp.bfloat16, jnp.float32
NT = (((1,), (1,)), ((), ()))
TN = (((0,), (0,)), ((), ()))


def _ln(x):
    m = jnp.mean(x, axis=-1, keepdims=True)
    c = x - m
    v = jnp.mean(c * c, axis=-1, keepdims=True)
    return c * lax.rsqrt(v + 1e-5)


def _gelu(x):
    return 0.5 * x * (1.0 + jnp.tanh(0.7978845608028654 * (x + 0.044715 * (x * x * x))))


def _kernel(x_hbm, wqkv_hbm, wo_hbm, w1_hbm, b1_hbm, w2_hbm, b2_hbm, o_hbm,
            x_ref, wqkv_ref, wo_ref, w1_ref, b1_ref, w2_ref, b2_ref, o_ref, sems, xs, q_s, k_s, vt_s, ot_s, s0_s, s1_s, s2_s, p0_s, p1_s, p2_s):
    NB = S // R

    def x_cp(r):
        return pltpu.make_async_copy(x_hbm.at[pl.ds(r * R, R)], x_ref.at[pl.ds(r * R, R)], sems.at[r])

    def o_cp(r):
        return pltpu.make_async_copy(o_ref.at[pl.ds(r * R, R)], o_hbm.at[pl.ds(r * R, R)], sems.at[NB + r])

    w_cp = [pltpu.make_async_copy(a, b, sems.at[2 * NB + i]) for i, (a, b) in enumerate(
        ((wqkv_hbm, wqkv_ref), (wo_hbm, wo_ref), (w1_hbm, w1_ref), (w2_hbm, w2_ref), (b1_hbm, b1_ref), (b2_hbm, b2_ref)))]
    x_cp(0).start()
    w_cp[0].start()
    for r in range(1, NB):
        x_cp(r).start()
    for c in w_cp[1:]:
        c.start()
    k_s[:, 0:W, :] = jnp.where(lax.broadcasted_iota(jnp.int32, (8, W, 128), 2) == 80, -1e30, 0.0).astype(BF)
    vt_s[:, 0:W // 128] = jnp.zeros((H, W // 128, 32, 128), BF)
    qscale = DH ** -0.5 * 1.4426950408889634

    def qkv_blk(r, l):
        r0 = pl.multiple_of(r * R, R)

        @pl.when(l == 0)
        def _():
            x_cp(r).wait()
            xs[pl.ds(r0, R), :] = x_ref[pl.ds(r0, R), :].astype(F32)

        xn = _ln(xs[pl.ds(r0, R), :]).astype(BF)
        q = jnp.dot(xn, wqkv_ref[:, 0:D], preferred_element_type=F32) * qscale
        k = jnp.dot(xn, wqkv_ref[:, D:2 * D], preferred_element_type=F32)
        v = jnp.dot(xn, wqkv_ref[:, 2 * D:3 * D], preferred_element_type=F32)
        lane = lax.broadcasted_iota(jnp.int32, (R, 128), 1)
        qT = q.T
        qfill = jnp.where(lax.broadcasted_iota(jnp.int32, (KC - 80, R), 0) == 0, 1.0, 0.0)
        for g in range(8):
            lo = min(80 * g, D - 128)
            kt = k[:, lo:lo + 128]
            if lo != 80 * g:
                kt = pltpu.roll(kt, 128 - (80 * g - lo), 1)
            qg = jnp.concatenate([qT[80 * g:80 * g + 80], qfill], axis=0).astype(BF)
            for c in range(R // 128):
                q_s[g, r * (R // 128) + c] = qg[:, c * 128:(c + 1) * 128]
            k_s[g, pl.ds(W + r0, R), :] = jnp.where(lane == 80, 0.0, kt).astype(BF)
        vt = v.T
        row = lax.broadcasted_iota(jnp.int32, (32, R), 0)
        fill = jnp.where(row == DH, 1.0, 0.0)
        for h in range(H):
            lo = min(h * DH, D - 32)
            blk = vt[lo:lo + 32, :]
            if lo != h * DH:
                blk = jnp.concatenate([blk[32 - DH:, :], blk[:32 - DH, :]], axis=0)
            blk = jnp.where(row < DH, blk, fill).astype(BF)
            for c in range(R // 128):
                vt_s[h, W // 128 + r * (R // 128) + c] = blk[:, c * 128:(c + 1) * 128]
        return l

    def st_qk(u, s_ref):
        qb, g = u // 8, u % 8
        q0 = pl.multiple_of(qb * 128, 128)
        rw = lax.broadcasted_iota(jnp.int32, (KC // 2, 128), 0)
        qi = q_s.bitcast(jnp.int32)[g, qb]
        qm = jnp.concatenate(
            [pltpu.bitcast(jnp.where(((rw >= 10 * j) & (rw < 10 * j + 10)) | (rw == 40), qi, 0), BF) for j in range(4)], axis=1)
        kk = pltpu.bitcast(k_s.bitcast(jnp.int32)[g, pl.ds(pl.multiple_of(qb * 64, 64), 192), :], BF)
        s_ref[...] = jnp.dot(kk[:, 0:KC], qm, preferred_element_type=F32)

    def st_sm(s_ref, p_ref):
        tri = lax.broadcasted_iota(jnp.int32, (128, 128), 0) <= lax.broadcasted_iota(jnp.int32, (128, 128), 1)
        for j in range(4):
            c = slice(j * 128, (j + 1) * 128)
            t = jnp.where(tri, s_ref[256:384, c], s_ref[0:128, c])
            s1 = s_ref[128:256, c]
            m = jnp.max(jnp.maximum(t, s1), axis=0, keepdims=True)
            pt = jnp.exp2(t - m)
            p_ref[j, 0:128, :] = jnp.where(tri, 0.0, pt).astype(BF)
            p_ref[j, 128:256, :] = jnp.exp2(s1 - m).astype(BF)
            p_ref[j, 256:384, :] = jnp.where(tri, pt, 0.0).astype(BF)

    def st_pv(u, p_ref):
        qb, g = u // 8, u % 8
        q0 = pl.multiple_of(qb * 128, 128)
        outs = []
        for j in range(4):
            vv = jnp.concatenate([pltpu.bitcast(vt_s.bitcast(jnp.int32)[g * 4 + j, qb + c], BF) for c in range(3)], axis=1)
            o = jnp.dot(vv, pltpu.bitcast(p_ref.bitcast(jnp.int32)[j], BF), preferred_element_type=F32)
            outs.append((o[0:24] * (1.0 / o[DH:DH + 1]))[0:DH])
        ot_s[pl.ds(pl.multiple_of(g * 80, 8), 80), pl.ds(q0, 128)] = jnp.concatenate(outs, axis=0)

    def attention():
        U = (S // 128) * 8
        sb, pb = (s0_s, s1_s, s2_s), (p0_s, p1_s, p2_s)
        st_qk(0, sb[0])
        st_qk(1, sb[1])
        st_sm(sb[0], pb[0])

        def body(i, _):
            for t in range(UNR):
                u = 2 + UNR * i + t
                st_qk(u, sb[(2 + t) % 3])
                st_sm(sb[(1 + t) % 3], pb[(1 + t) % 3])
                st_pv(u - 2, pb[t % 3])
            return 0
        lax.fori_loop(0, (U - 2) // UNR, body, 0)
        st_sm(sb[(U - 1) % 3], pb[(U - 1) % 3])
        st_pv(U - 2, pb[(U - 2) % 3])
        st_pv(U - 1, pb[(U - 1) % 3])

    def ffn_blk(r, l):
        r0 = pl.multiple_of(r * R, R)
        ot = ot_s[:, pl.ds(r0, R)].astype(BF)
        x = xs[pl.ds(r0, R), :] + lax.dot_general(ot, wo_ref[...], TN, preferred_element_type=F32)
        xn = _ln(x).astype(BF)
        h = lax.dot_general(xn, w1_ref[...], NT, preferred_element_type=F32) + b1_ref[...].astype(F32)
        h = _gelu(h).astype(BF)
        x = x + jnp.dot(h, w2_ref[...], preferred_element_type=F32) + b2_ref[...].astype(F32)
        xs[pl.ds(r0, R), :] = x
        o_ref[pl.ds(r0, R), :] = x.astype(BF)

        @pl.when(l == 1)
        def _():
            o_cp(r).start()
        return l

    def layer(l, _):
        lax.fori_loop(0, NB, qkv_blk, l)
        attention()

        @pl.when(l == 0)
        def _():
            for c in w_cp[1:]:
                c.wait()
        lax.fori_loop(0, NB, ffn_blk, l)
        return 0

    w_cp[0].wait()
    lax.fori_loop(0, 2, layer, 0)
    for r in range(NB):
        o_cp(r).wait()


@jax.jit
def pallas_interleave_layers__sliding_block__dense_activation_gelu__prompt_kernel(A_x, A_wqkv, A_wo, B_x, B_w1, B_b1, B_w2, B_b2):
    out = pl.pallas_call(
        _kernel,
        out_shape=jax.ShapeDtypeStruct((S, D), BF),
        in_specs=[pl.BlockSpec(memory_space=pl.ANY)] * 7,
        out_specs=pl.BlockSpec(memory_space=pl.ANY),
        scratch_shapes=[
            pltpu.VMEM((S, D), BF), pltpu.VMEM((D, 3 * D), BF), pltpu.VMEM((D, D), BF), pltpu.VMEM((F, D), BF),
            pltpu.VMEM((1, F), BF), pltpu.VMEM((F, D), BF), pltpu.VMEM((1, D), BF), pltpu.VMEM((S, D), BF),
            pltpu.SemaphoreType.DMA((2 * (S // R) + 6,)),
            pltpu.VMEM((S, D), F32),
            pltpu.VMEM((8, S // 128, KC, 128), BF),
            pltpu.VMEM((8, S + W, 128), BF),
            pltpu.VMEM((H, (S + W) // 128, 32, 128), BF),
            pltpu.VMEM((D, S), F32),
            pltpu.VMEM((384, 512), F32),
            pltpu.VMEM((384, 512), F32),
            pltpu.VMEM((384, 512), F32),
            pltpu.VMEM((4, 384, 128), BF),
            pltpu.VMEM((4, 384, 128), BF),
            pltpu.VMEM((4, 384, 128), BF),
        ],
        compiler_params=pltpu.CompilerParams(vmem_limit_bytes=100 * 1024 * 1024),
    )(A_x.reshape(S, D), A_wqkv, A_wo, B_w1.T, B_b1.reshape(1, F), B_w2, B_b2.reshape(1, D))
    return out.reshape(1, S, D)
```

```python
import jax
import jax.numpy as jnp
from jax import lax
import jax.experimental.pallas as pl
import jax.experimental.pallas.tpu as pltpu

S, D, H, DH, W, F = 2048, 640, 32, 20, 256, 1728
BASES = (0, 120, 240, 360, 480, 512)
R = 512
UNR = 24
GU = 1
LS = 2
LP = 3
GQ = 1
GF = 1
KC = 96
BF, F32 = jnp.bfloat16, jnp.float32
NT = (((1,), (1,)), ((), ()))
TN = (((0,), (0,)), ((), ()))


def _ln(x):
    m = jnp.mean(x, axis=-1, keepdims=True)
    c = x - m
    v = jnp.mean(c * c, axis=-1, keepdims=True)
    return c * lax.rsqrt(v + 1e-5)


def _gelu(x):
    return 0.5 * x * (1.0 + jnp.tanh(0.7978845608028654 * (x + 0.044715 * (x * x * x))))


def _kernel(x_hbm, wqkv_hbm, wo_hbm, w1_hbm, b1_hbm, w2_hbm, b2_hbm, o_hbm,
            x_ref, wqkv_ref, wo_ref, w1_ref, b1_ref, w2_ref, b2_ref, o_ref, sems, xs, xa_s, xb_s, q_s, k_s, vt_s, ot_s, s0_s, s1_s, s2_s, s3_s, p0_s, p1_s, p2_s, p3_s):
    NB = S // R

    def x_cp(r):
        return pltpu.make_async_copy(x_hbm.at[pl.ds(r * R, R)], x_ref.at[pl.ds(r * R, R)], sems.at[r])

    def o_cp(r):
        return pltpu.make_async_copy(o_ref.at[pl.ds(r * R, R)], o_hbm.at[pl.ds(r * R, R)], sems.at[NB + r])

    w_cp = [pltpu.make_async_copy(a, b, sems.at[2 * NB + i]) for i, (a, b) in enumerate(
        ((wqkv_hbm, wqkv_ref), (wo_hbm, wo_ref), (w1_hbm, w1_ref), (w2_hbm, w2_ref)))]
    x_cp(0).start()
    w_cp[0].start()
    k_s[:, 0:W, :] = jnp.where(lax.broadcasted_iota(jnp.int32, (8, W, 128), 2) == 80, -1e30, 0.0).astype(BF)
    vt_s[:, 0:W // 128] = jnp.zeros((H, W // 128, 32, 128), BF)
    qscale = DH ** -0.5 * 1.4426950408889634

    def ln_blk(r, dst):
        dst[...] = _ln(xs[pl.ds(pl.multiple_of(r * R, R), R), :]).astype(BF)

    def x_in(r):
        x_cp(r).wait()
        xs[r * R:(r + 1) * R, :] = x_ref[r * R:(r + 1) * R, :].astype(F32)

    def qkv_blk(r, xn_ref):
        r0 = pl.multiple_of(r * R, R)
        xn = xn_ref[...]
        v = jnp.dot(xn, wqkv_ref[:, 2 * D:3 * D], preferred_element_type=F32)
        vt = v.T
        row = lax.broadcasted_iota(jnp.int32, (32, R), 0)
        fill = jnp.where(row == DH, 1.0, 0.0)
        for h in range(H):
            lo = min(h * DH, D - 32)
            blk = vt[lo:lo + 32, :]
            if lo != h * DH:
                blk = jnp.concatenate([blk[32 - DH:, :], blk[:32 - DH, :]], axis=0)
            blk = jnp.where(row < DH, blk, fill).astype(BF)
            for c in range(R // 128):
                vt_s[h, W // 128 + r * (R // 128) + c] = blk[:, c * 128:(c + 1) * 128]
        q = jnp.dot(xn, wqkv_ref[:, 0:D], preferred_element_type=F32) * qscale
        qT = q.T
        qfill = jnp.where(lax.broadcasted_iota(jnp.int32, (KC - 80, R), 0) == 0, 1.0, 0.0)
        for g in range(8):
            qg = jnp.concatenate([qT[80 * g:80 * g + 80], qfill], axis=0).astype(BF)
            for c in range(R // 128):
                q_s[g, r * (R // 128) + c] = qg[:, c * 128:(c + 1) * 128]
        k = jnp.dot(xn, wqkv_ref[:, D:2 * D], preferred_element_type=F32)
        lane = lax.broadcasted_iota(jnp.int32, (R, 128), 1)
        for g in range(8):
            lo = min(80 * g, D - 128)
            kt = k[:, lo:lo + 128]
            if lo != 80 * g:
                kt = pltpu.roll(kt, 128 - (80 * g - lo), 1)
            k_s[g, pl.ds(W + r0, R), :] = jnp.where(lane == 80, 0.0, kt).astype(BF)

    def st_qk(u, s_ref):
        for e in range(GU):
            st_qk1(u // (8 // GU), (u % (8 // GU)) * GU + e, s_ref, e)

    def st_qk1(qb, g, s_ref, e):
        q0 = pl.multiple_of(qb * 128, 128)
        rw = lax.broadcasted_iota(jnp.int32, (KC // 2, 128), 0)
        qi = q_s.bitcast(jnp.int32)[g, qb]
        qm = jnp.concatenate(
            [pltpu.bitcast(jnp.where(((rw >= 10 * j) & (rw < 10 * j + 10)) | (rw == 40), qi, 0), BF) for j in range(4)], axis=1)
        kk = pltpu.bitcast(k_s.bitcast(jnp.int32)[g, pl.ds(pl.multiple_of(qb * 64, 64), 192), :], BF)
        s_ref[:, e * 512:(e + 1) * 512] = jnp.dot(kk[:, 0:KC], qm, preferred_element_type=F32)

    def st_sm(s_ref, p_ref):
        tri = lax.broadcasted_iota(jnp.int32, (128, 128), 0) <= lax.broadcasted_iota(jnp.int32, (128, 128), 1)
        for j in range(4 * GU):
            c = slice(j * 128, (j + 1) * 128)
            t = jnp.where(tri, s_ref[256:384, c], s_ref[0:128, c])
            s1 = s_ref[128:256, c]
            m = jnp.max(jnp.maximum(t, s1), axis=0, keepdims=True)
            pt = jnp.exp2(t - m)
            p_ref[j, 0:128, :] = jnp.where(tri, 0.0, pt).astype(BF)
            p_ref[j, 128:256, :] = jnp.exp2(s1 - m).astype(BF)
            p_ref[j, 256:384, :] = jnp.where(tri, pt, 0.0).astype(BF)

    def st_pv(u, p_ref):
        for e in range(GU):
            st_pv1(u // (8 // GU), (u % (8 // GU)) * GU + e, p_ref, e)

    def st_pv1(qb, g, p_ref, e):
        q0 = pl.multiple_of(qb * 128, 128)
        outs = []
        for j in range(4):
            vv = jnp.concatenate([pltpu.bitcast(vt_s.bitcast(jnp.int32)[g * 4 + j, qb + c], BF) for c in range(3)], axis=1)
            o = jnp.dot(vv, pltpu.bitcast(p_ref.bitcast(jnp.int32)[4 * e + j], BF), preferred_element_type=F32)
            outs.append((o[0:24] * (1.0 / o[DH:DH + 1]))[0:DH])
        ot_s[pl.ds(pl.multiple_of(g * 80, 8), 80), pl.ds(q0, 128)] = jnp.concatenate(outs, axis=0)

    def attention():
        U = (S // 128) * 8 // GU
        sb, pb = (s0_s, s1_s, s2_s, s3_s), (p0_s, p1_s, p2_s, p3_s)

        def step(u, t):
            if not isinstance(u, int) or u < U:
                st_qk(u, sb[t % 4])
            if not isinstance(u, int) or LS <= u < U + LS:
                st_sm(sb[(t - LS) % 4], pb[(t - LS) % 4])
            if not isinstance(u, int) or u >= LP:
                st_pv(u - LP, pb[(t - LP) % 4])

        def body(i, _):
            for t in range(UNR):
                step(LP + UNR * i + t, LP + t)
            return 0
        nit = (U - LP) // UNR
        for u in range(LP):
            step(u, u)
        lax.fori_loop(0, nit, body, 0)
        for u in range(LP + nit * UNR, U + LP):
            step(u, u)

    def ffn_blk(r, l):
        r0 = pl.multiple_of(r * R, R)
        ot = ot_s[:, pl.ds(r0, R)].astype(BF)
        x = xs[pl.ds(r0, R), :] + lax.dot_general(ot, wo_ref[...], TN, preferred_element_type=F32)
        xn = _ln(x).astype(BF)
        h = lax.dot_general(xn, w1_ref[...], NT, preferred_element_type=F32) + b1_hbm[...].astype(F32).reshape(1, F)
        h = _gelu(h).astype(BF)
        x = x + jnp.dot(h, w2_ref[...], preferred_element_type=F32) + b2_hbm[...].astype(F32).reshape(1, D)
        xs[pl.ds(r0, R), :] = x
        o_ref[pl.ds(r0, R), :] = x.astype(BF)
        return l

    def qkv_it(i, l):
        for ii in range(NB // 2):
            @pl.when(jnp.logical_and(l == 0, i == ii))
            def _():
                for r in range(2 * ii + 1, min(2 * ii + 3, NB)):
                    x_in(r)
        ln_blk(2 * i + 1, xb_s)
        qkv_blk(2 * i, xa_s)
        ln_blk(jnp.minimum(2 * i + 2, NB - 1), xa_s)
        qkv_blk(2 * i + 1, xb_s)
        return l

    def ffn_it(i, l):
        @pl.when(jnp.logical_and(l == 1, i > 0))
        def _():
            for t in range(GF):
                o_cp((i - 1) * GF + t).start()
        for t in range(GF):
            ffn_blk(i * GF + t, l)
        return l

    def layer(l, _):
        @pl.when(l == 0)
        def _():
            x_in(0)
        ln_blk(0, xa_s)
        lax.fori_loop(0, NB // 2, qkv_it, l)

        @pl.when(l == 0)
        def _():
            for c in w_cp[1:]:
                c.start()
        attention()

        @pl.when(l == 0)
        def _():
            for c in w_cp[1:]:
                c.wait()
        lax.fori_loop(0, NB // GF, ffn_it, l)
        return 0

    w_cp[0].wait()
    for r in range(1, NB):
        x_cp(r).start()
    lax.fori_loop(0, 2, layer, 0)
    for r in range(NB - GF, NB):
        o_cp(r).start()
    for r in range(NB):
        o_cp(r).wait()


@jax.jit
def pallas_interleave_layers__sliding_block__dense_activation_gelu__prompt_kernel(A_x, A_wqkv, A_wo, B_x, B_w1, B_b1, B_w2, B_b2):
    out = pl.pallas_call(
        _kernel,
        out_shape=jax.ShapeDtypeStruct((S, D), BF),
        in_specs=[pl.BlockSpec(memory_space=m) for m in (pl.ANY,) * 4 + (pltpu.VMEM, pl.ANY, pltpu.VMEM)],
        out_specs=pl.BlockSpec(memory_space=pl.ANY),
        scratch_shapes=[
            pltpu.VMEM((S, D), BF), pltpu.VMEM((D, 3 * D), BF), pltpu.VMEM((D, D), BF), pltpu.VMEM((F, D), BF),
            pltpu.VMEM((1, F), BF), pltpu.VMEM((F, D), BF), pltpu.VMEM((1, D), BF), pltpu.VMEM((S, D), BF),
            pltpu.SemaphoreType.DMA((2 * (S // R) + 6,)),
            pltpu.VMEM((S, D), F32), pltpu.VMEM((R, D), BF), pltpu.VMEM((R, D), BF),
            pltpu.VMEM((8, S // 128, KC, 128), BF),
            pltpu.VMEM((8, S + W, 128), BF),
            pltpu.VMEM((H, (S + W) // 128, 32, 128), BF),
            pltpu.VMEM((D, S), F32),
            pltpu.VMEM((384, 512 * GU), F32),
            pltpu.VMEM((384, 512 * GU), F32),
            pltpu.VMEM((384, 512 * GU), F32),
            pltpu.VMEM((384, 512 * GU), F32),
            pltpu.VMEM((4 * GU, 384, 128), BF),
            pltpu.VMEM((4 * GU, 384, 128), BF),
            pltpu.VMEM((4 * GU, 384, 128), BF),
            pltpu.VMEM((4 * GU, 384, 128), BF),
        ],
        compiler_params=pltpu.CompilerParams(vmem_limit_bytes=100 * 1024 * 1024, flags={'XLA_TPU_EVENLY_DISTRIBUTE_CRITICAL_NODES': True}),
    )(A_x.reshape(S, D), A_wqkv, A_wo, B_w1.T, B_b1, B_w2, B_b2)
    return out.reshape(1, S, D)
```

```python
import jax
import jax.numpy as jnp
from jax import lax
import jax.experimental.pallas as pl
import jax.experimental.pallas.tpu as pltpu

S, D, H, DH, W, F = 2048, 640, 32, 20, 256, 1728
R = 512
UNR = 24
GU = 1
LS = 2
LP = 3
GQ = 1
GF = 1
KC = 96
BF, F32 = jnp.bfloat16, jnp.float32
NT = (((1,), (1,)), ((), ()))
TN = (((0,), (0,)), ((), ()))


def _ln(x):
    m = jnp.mean(x, axis=-1, keepdims=True)
    c = x - m
    v = jnp.mean(c * c, axis=-1, keepdims=True)
    return c * lax.rsqrt(v + 1e-5)


def _gelu(x):
    return 0.5 * x * (1.0 + jnp.tanh(0.7978845608028654 * (x + 0.044715 * (x * x * x))))


def _kernel(x_hbm, wqkv_hbm, wo_hbm, w1_hbm, b1_hbm, w2_hbm, b2_hbm, o_hbm,
            x_ref, wqkv_ref, wo_ref, w1_ref, w2_ref, o_ref, sems, xs, xa_s, xb_s, q_s, k_s, vt_s, ot_s, s0_s, s1_s, s2_s, s3_s, p0_s, p1_s, p2_s, p3_s):
    NB = S // R

    def x_cp(r):
        return pltpu.make_async_copy(x_hbm.at[pl.ds(r * R, R)], x_ref.at[pl.ds(r * R, R)], sems.at[r])

    def o_cp(r):
        return pltpu.make_async_copy(o_ref.at[pl.ds(r * R, R)], o_hbm.at[pl.ds(r * R, R)], sems.at[NB + r])

    w_cp = [pltpu.make_async_copy(a, b, sems.at[2 * NB + i]) for i, (a, b) in enumerate(
        ((wqkv_hbm, wqkv_ref), (wo_hbm, wo_ref), (w1_hbm, w1_ref), (w2_hbm, w2_ref)))]
    x_cp(0).start()
    w_cp[0].start()
    k_s[:, 0:W, :] = jnp.where(lax.broadcasted_iota(jnp.int32, (8, W, 128), 2) == 80, -1e30, 0.0).astype(BF)
    vt_s[:, 0:W // 128] = jnp.zeros((H, W // 128, 32, 128), BF)
    qscale = DH ** -0.5 * 1.4426950408889634

    def ln_blk(r, dst):
        dst[...] = _ln(xs[pl.ds(pl.multiple_of(r * R, R), R), :]).astype(BF)

    def x_in(r):
        x_cp(r).wait()
        xs[r * R:(r + 1) * R, :] = x_ref[r * R:(r + 1) * R, :].astype(F32)

    def qkv_blk(r, xn_ref):
        r0 = pl.multiple_of(r * R, R)
        xn = xn_ref[...]
        v = jnp.dot(xn, wqkv_ref[:, 2 * D:3 * D], preferred_element_type=F32)
        vt = v.T
        row = lax.broadcasted_iota(jnp.int32, (32, R), 0)
        fill = jnp.where(row == DH, 1.0, 0.0)
        for h in range(H):
            lo = min(h * DH, D - 32)
            blk = vt[lo:lo + 32, :]
            if lo != h * DH:
                blk = jnp.concatenate([blk[32 - DH:, :], blk[:32 - DH, :]], axis=0)
            blk = jnp.where(row < DH, blk, fill).astype(BF)
            for c in range(R // 128):
                vt_s[h, W // 128 + r * (R // 128) + c] = blk[:, c * 128:(c + 1) * 128]
        q = jnp.dot(xn, wqkv_ref[:, 0:D], preferred_element_type=F32) * qscale
        qT = q.T
        qfill = jnp.where(lax.broadcasted_iota(jnp.int32, (KC - 80, R), 0) == 0, 1.0, 0.0)
        for g in range(8):
            qg = jnp.concatenate([qT[80 * g:80 * g + 80], qfill], axis=0).astype(BF)
            for c in range(R // 128):
                q_s[g, r * (R // 128) + c] = qg[:, c * 128:(c + 1) * 128]
        k = jnp.dot(xn, wqkv_ref[:, D:2 * D], preferred_element_type=F32)
        lane = lax.broadcasted_iota(jnp.int32, (R, 128), 1)
        for g in range(8):
            lo = min(80 * g, D - 128)
            kt = k[:, lo:lo + 128]
            if lo != 80 * g:
                kt = pltpu.roll(kt, 128 - (80 * g - lo), 1)
            k_s[g, pl.ds(W + r0, R), :] = jnp.where(lane == 80, 0.0, kt).astype(BF)

    def st_qk(u, s_ref):
        for e in range(GU):
            st_qk1(u // (8 // GU), (u % (8 // GU)) * GU + e, s_ref, e)

    def st_qk1(qb, g, s_ref, e):
        q0 = pl.multiple_of(qb * 128, 128)
        rw = lax.broadcasted_iota(jnp.int32, (KC // 2, 128), 0)
        qi = q_s.bitcast(jnp.int32)[g, qb]
        qm = jnp.concatenate(
            [pltpu.bitcast(jnp.where(((rw >= 10 * j) & (rw < 10 * j + 10)) | (rw == 40), qi, 0), BF) for j in range(4)], axis=1)
        kk = pltpu.bitcast(k_s.bitcast(jnp.int32)[g, pl.ds(pl.multiple_of(qb * 64, 64), 192), :], BF)
        s_ref[:, e * 512:(e + 1) * 512] = jnp.dot(kk[:, 0:KC], qm, preferred_element_type=F32)

    def st_sm(s_ref, p_ref):
        tri = lax.broadcasted_iota(jnp.int32, (128, 128), 0) <= lax.broadcasted_iota(jnp.int32, (128, 128), 1)
        for j in range(4 * GU):
            c = slice(j * 128, (j + 1) * 128)
            t = jnp.where(tri, s_ref[256:384, c], s_ref[0:128, c])
            s1 = s_ref[128:256, c]
            m = jnp.max(jnp.maximum(t, s1), axis=0, keepdims=True)
            pt = jnp.exp2(t - m)
            p_ref[j, 0:128, :] = jnp.where(tri, 0.0, pt).astype(BF)
            p_ref[j, 128:256, :] = jnp.exp2(s1 - m).astype(BF)
            p_ref[j, 256:384, :] = jnp.where(tri, pt, 0.0).astype(BF)

    def st_pv(u, p_ref):
        for e in range(GU):
            st_pv1(u // (8 // GU), (u % (8 // GU)) * GU + e, p_ref, e)

    def st_pv1(qb, g, p_ref, e):
        q0 = pl.multiple_of(qb * 128, 128)
        outs = []
        for j in range(4):
            vv = jnp.concatenate([pltpu.bitcast(vt_s.bitcast(jnp.int32)[g * 4 + j, qb + c], BF) for c in range(3)], axis=1)
            o = jnp.dot(vv, pltpu.bitcast(p_ref.bitcast(jnp.int32)[4 * e + j], BF), preferred_element_type=F32)
            outs.append((o[0:24] * (1.0 / o[DH:DH + 1]))[0:DH])
        ot_s[pl.ds(pl.multiple_of(g * 80, 8), 80), pl.ds(q0, 128)] = jnp.concatenate(outs, axis=0)

    def attention():
        U = (S // 128) * 8 // GU
        sb, pb = (s0_s, s1_s, s2_s, s3_s), (p0_s, p1_s, p2_s, p3_s)

        def step(u, t):
            if not isinstance(u, int) or u < U:
                st_qk(u, sb[t % 4])
            if not isinstance(u, int) or LS <= u < U + LS:
                st_sm(sb[(t - LS) % 4], pb[(t - LS) % 4])
            if not isinstance(u, int) or u >= LP:
                st_pv(u - LP, pb[(t - LP) % 4])

        def body(i, _):
            for t in range(UNR):
                step(LP + UNR * i + t, LP + t)
            return 0
        nit = (U - LP) // UNR
        for u in range(LP):
            step(u, u)
        lax.fori_loop(0, nit, body, 0)
        for u in range(LP + nit * UNR, U + LP):
            step(u, u)

    def ffn_blk(r, l):
        r0 = pl.multiple_of(r * R, R)
        ot = ot_s[:, pl.ds(r0, R)].astype(BF)
        x = xs[pl.ds(r0, R), :] + lax.dot_general(ot, wo_ref[...], TN, preferred_element_type=F32)
        xn = _ln(x).astype(BF)
        h = lax.dot_general(xn, w1_ref[...], NT, preferred_element_type=F32) + b1_hbm[...].astype(F32).reshape(1, F)
        h = _gelu(h).astype(BF)
        x = x + jnp.dot(h, w2_ref[...], preferred_element_type=F32) + b2_hbm[...].astype(F32).reshape(1, D)
        xs[pl.ds(r0, R), :] = x
        o_ref[pl.ds(r0, R), :] = x.astype(BF)
        return l

    def qkv_it(i, l):
        for ii in range(NB // 2):
            @pl.when(jnp.logical_and(l == 0, i == ii))
            def _():
                for r in range(2 * ii + 1, min(2 * ii + 3, NB)):
                    x_in(r)
        ln_blk(2 * i + 1, xb_s)
        qkv_blk(2 * i, xa_s)
        ln_blk(jnp.minimum(2 * i + 2, NB - 1), xa_s)
        qkv_blk(2 * i + 1, xb_s)
        return l

    def ffn_it(i, l):
        @pl.when(jnp.logical_and(l == 1, i > 0))
        def _():
            for t in range(GF):
                o_cp((i - 1) * GF + t).start()
        for t in range(GF):
            ffn_blk(i * GF + t, l)
        return l

    def layer(l, _):
        @pl.when(l == 0)
        def _():
            x_in(0)
        ln_blk(0, xa_s)
        lax.fori_loop(0, NB // 2, qkv_it, l)

        @pl.when(l == 0)
        def _():
            for c in w_cp[1:]:
                c.start()
        attention()

        @pl.when(l == 0)
        def _():
            for c in w_cp[1:]:
                c.wait()
        lax.fori_loop(0, NB // GF, ffn_it, l)
        return 0

    w_cp[0].wait()
    for r in range(1, NB):
        x_cp(r).start()
    lax.fori_loop(0, 2, layer, 0)
    for r in range(NB - GF, NB):
        o_cp(r).start()
    for r in range(NB):
        o_cp(r).wait()


@jax.jit
def pallas_interleave_layers__sliding_block__dense_activation_gelu__prompt_kernel(A_x, A_wqkv, A_wo, B_x, B_w1, B_b1, B_w2, B_b2):
    out = pl.pallas_call(
        _kernel,
        out_shape=jax.ShapeDtypeStruct((S, D), BF),
        in_specs=[pl.BlockSpec(memory_space=m) for m in (pl.ANY,) * 4 + (pltpu.VMEM, pl.ANY, pltpu.VMEM)],
        out_specs=pl.BlockSpec(memory_space=pl.ANY),
        scratch_shapes=[
            pltpu.VMEM((S, D), BF), pltpu.VMEM((D, 3 * D), BF), pltpu.VMEM((D, D), BF), pltpu.VMEM((F, D), BF),
            pltpu.VMEM((F, D), BF), pltpu.VMEM((S, D), BF),
            pltpu.SemaphoreType.DMA((2 * (S // R) + 4,)),
            pltpu.VMEM((S, D), F32), pltpu.VMEM((R, D), BF), pltpu.VMEM((R, D), BF),
            pltpu.VMEM((8, S // 128, KC, 128), BF),
            pltpu.VMEM((8, S + W, 128), BF),
            pltpu.VMEM((H, (S + W) // 128, 32, 128), BF),
            pltpu.VMEM((D, S), F32),
            pltpu.VMEM((384, 512 * GU), F32),
            pltpu.VMEM((384, 512 * GU), F32),
            pltpu.VMEM((384, 512 * GU), F32),
            pltpu.VMEM((384, 512 * GU), F32),
            pltpu.VMEM((4 * GU, 384, 128), BF),
            pltpu.VMEM((4 * GU, 384, 128), BF),
            pltpu.VMEM((4 * GU, 384, 128), BF),
            pltpu.VMEM((4 * GU, 384, 128), BF),
        ],
        compiler_params=pltpu.CompilerParams(vmem_limit_bytes=100 * 1024 * 1024, flags={'XLA_TPU_EVENLY_DISTRIBUTE_CRITICAL_NODES': True}),
    )(A_x.reshape(S, D), A_wqkv, A_wo, B_w1.T, B_b1, B_w2, B_b2)
    return out.reshape(1, S, D)
```

```python
import jax
import jax.numpy as jnp
from jax import lax
import jax.experimental.pallas as pl
import jax.experimental.pallas.tpu as pltpu

S, D, H, DH, W, F = 2048, 640, 32, 20, 256, 1728
R = 512
UNR = 24
GU = 1
LS = 2
LP = 3
GQ = 1
GF = 1
KC = 96
BF, F32 = jnp.bfloat16, jnp.float32
NT = (((1,), (1,)), ((), ()))
TN = (((0,), (0,)), ((), ()))


def _ln(x):
    m = jnp.mean(x, axis=-1, keepdims=True)
    c = x - m
    v = jnp.mean(c * c, axis=-1, keepdims=True)
    return c * lax.rsqrt(v + 1e-5)


def _gelu(x):
    return 0.5 * x * (1.0 + jnp.tanh(0.7978845608028654 * (x + 0.044715 * (x * x * x))))


def _kernel(x_hbm, wqkv_hbm, wo_hbm, w1_hbm, b1_hbm, w2_hbm, b2_hbm, o_hbm,
            x_ref, wqkv_ref, wo_ref, w1_ref, w2_ref, o_ref, sems, xs, xn_s, q_s, k_s, vt_s, ot_s, s0_s, s1_s, s2_s, s3_s, p0_s, p1_s, p2_s, p3_s):
    NB = S // R

    def x_cp(r):
        return pltpu.make_async_copy(x_hbm.at[pl.ds(r * R, R)], x_ref.at[pl.ds(r * R, R)], sems.at[r])

    def o_cp(r):
        return pltpu.make_async_copy(o_ref.at[pl.ds(r * R, R)], o_hbm.at[pl.ds(r * R, R)], sems.at[NB + r])

    w_cp = [pltpu.make_async_copy(a, b, sems.at[2 * NB + i]) for i, (a, b) in enumerate(
        ((wo_hbm, wo_ref), (w1_hbm, w1_ref), (w2_hbm, w2_ref)))]
    wq_cp = [pltpu.make_async_copy(wqkv_hbm.at[:, pl.ds(j * D, D)], wqkv_ref.at[:, pl.ds(j * D, D)],
                                   sems.at[2 * NB + 4 + j]) for j in (2, 0, 1)]
    x_cp(0).start()
    wq_cp[0].start()
    k_s[:, 0:W, :] = jnp.where(lax.broadcasted_iota(jnp.int32, (8, W, 128), 2) == 80, -1e30, 0.0).astype(BF)
    vt_s[:, 0:W // 128] = jnp.zeros((H, W // 128, 32, 128), BF)
    qscale = DH ** -0.5 * 1.4426950408889634

    def ln_blk(r, dst):
        dst[...] = _ln(xs[pl.ds(pl.multiple_of(r * R, R), R), :]).astype(BF)

    def x_in(r):
        x_cp(r).wait()
        xs[r * R:(r + 1) * R, :] = x_ref[r * R:(r + 1) * R, :].astype(F32)

    def v_blk(r):
        xn = xn_s[r * R:(r + 1) * R, :]
        v = jnp.dot(xn, wqkv_ref[:, 2 * D:3 * D], preferred_element_type=F32)
        vt = v.T
        row = lax.broadcasted_iota(jnp.int32, (32, R), 0)
        fill = jnp.where(row == DH, 1.0, 0.0)
        for h in range(H):
            lo = min(h * DH, D - 32)
            blk = vt[lo:lo + 32, :]
            if lo != h * DH:
                blk = jnp.concatenate([blk[32 - DH:, :], blk[:32 - DH, :]], axis=0)
            blk = jnp.where(row < DH, blk, fill).astype(BF)
            for c in range(R // 128):
                vt_s[h, W // 128 + r * (R // 128) + c] = blk[:, c * 128:(c + 1) * 128]

    def qk_blk(r, _):
        r0 = pl.multiple_of(r * R, R)
        xn = xn_s[pl.ds(r0, R), :]
        q = jnp.dot(xn, wqkv_ref[:, 0:D], preferred_element_type=F32) * qscale
        qT = q.T
        qfill = jnp.where(lax.broadcasted_iota(jnp.int32, (KC - 80, R), 0) == 0, 1.0, 0.0)
        for g in range(8):
            qg = jnp.concatenate([qT[80 * g:80 * g + 80], qfill], axis=0).astype(BF)
            for c in range(R // 128):
                q_s[g, r * (R // 128) + c] = qg[:, c * 128:(c + 1) * 128]
        k = jnp.dot(xn, wqkv_ref[:, D:2 * D], preferred_element_type=F32)
        lane = lax.broadcasted_iota(jnp.int32, (R, 128), 1)
        for g in range(8):
            lo = min(80 * g, D - 128)
            kt = k[:, lo:lo + 128]
            if lo != 80 * g:
                kt = pltpu.roll(kt, 128 - (80 * g - lo), 1)
            k_s[g, pl.ds(W + r0, R), :] = jnp.where(lane == 80, 0.0, kt).astype(BF)
        return 0

    def st_qk(u, s_ref):
        for e in range(GU):
            st_qk1(u // (8 // GU), (u % (8 // GU)) * GU + e, s_ref, e)

    def st_qk1(qb, g, s_ref, e):
        q0 = pl.multiple_of(qb * 128, 128)
        rw = lax.broadcasted_iota(jnp.int32, (KC // 2, 128), 0)
        lo = lax.broadcasted_iota(jnp.int32, (KC // 2, 128), 1) < 64
        qi = q_s.bitcast(jnp.int32)[g, qb]
        qr = pltpu.roll(qi, 64, 1)
        ki = k_s.bitcast(jnp.int32)
        for half in range(2):
            tiles = []
            for j in range(2):
                ma = ((rw >= 20 * j) & (rw < 20 * j + 10)) | (rw == 40)
                mb = ((rw >= 20 * j + 10) & (rw < 20 * j + 20)) | (rw == 40)
                ta, tb = jnp.where(ma, qi, 0), jnp.where(mb, qr, 0)
                tiles.append(pltpu.bitcast(jnp.where(lo, ta, tb) if half == 0 else jnp.where(lo, tb, ta), BF))
            kk = pltpu.bitcast(ki[g, pl.ds(pl.multiple_of(qb * 64 + 32 * half, 32), 160), :], BF)
            s_ref[:, half * 256:(half + 1) * 256] = jnp.dot(kk[:, 0:KC], jnp.concatenate(tiles, axis=1), preferred_element_type=F32)

    def st_sm(s_ref, p_ref):
        tri = lax.broadcasted_iota(jnp.int32, (64, 128), 0) <= (lax.broadcasted_iota(jnp.int32, (64, 128), 1) & 63)
        for j in range(4):
            c = slice(j * 128, (j + 1) * 128)
            t = jnp.where(tri, s_ref[256:320, c], s_ref[0:64, c])
            s1 = s_ref[64:256, c]
            m = jnp.maximum(jnp.max(t, axis=0, keepdims=True), jnp.max(s1, axis=0, keepdims=True))
            pt = jnp.exp2(t - m)
            p_ref[j, 0:64, :] = jnp.where(tri, 0.0, pt).astype(BF)
            p_ref[j, 64:256, :] = jnp.exp2(s1 - m).astype(BF)
            p_ref[j, 256:320, :] = jnp.where(tri, pt, 0.0).astype(BF)

    def st_pv(u, p_ref):
        for e in range(GU):
            st_pv1(u // (8 // GU), (u % (8 // GU)) * GU + e, p_ref, e)

    def st_pv1(qb, g, p_ref, e):
        q0 = pl.multiple_of(qb * 128, 128)
        outs = []
        pi = p_ref.bitcast(jnp.int32)
        lo = lax.broadcasted_iota(jnp.int32, (192, 128), 1) < 64
        zr = jnp.zeros((32, 128), jnp.int32)
        for j in range(2):
            p0 = jnp.concatenate([pi[j], zr], axis=0)
            p1 = jnp.concatenate([zr, pi[2 + j]], axis=0)
            for e2 in range(2):
                pp = jnp.where(lo, p0, p1) if e2 == 0 else jnp.where(lo, p1, p0)
                vv = jnp.concatenate([pltpu.bitcast(vt_s.bitcast(jnp.int32)[g * 4 + 2 * j + e2, qb + c], BF) for c in range(3)], axis=1)
                o = jnp.dot(vv, pltpu.bitcast(pp, BF), preferred_element_type=F32)
                o = (o[0:24] * (1.0 / o[DH:DH + 1]))[0:DH]
                outs.append(o if e2 == 0 else pltpu.roll(o, 64, 1))
        ot_s[pl.ds(pl.multiple_of(g * 80, 8), 80), pl.ds(q0, 128)] = jnp.concatenate(outs, axis=0)

    def attention():
        U = (S // 128) * 8 // GU
        sb, pb = (s0_s, s1_s, s2_s, s3_s), (p0_s, p1_s, p2_s, p3_s)

        def step(u, t):
            if not isinstance(u, int) or u < U:
                st_qk(u, sb[t % 4])
            if not isinstance(u, int) or LS <= u < U + LS:
                st_sm(sb[(t - LS) % 4], pb[(t - LS) % 4])
            if not isinstance(u, int) or u >= LP:
                st_pv(u - LP, pb[(t - LP) % 4])

        def body(i, _):
            for t in range(UNR):
                step(LP + UNR * i + t, LP + t)
            return 0
        nit = (U - LP) // UNR
        for u in range(LP):
            step(u, u)
        lax.fori_loop(0, nit, body, 0)
        for u in range(LP + nit * UNR, U + LP):
            step(u, u)

    def ffn_blk(r, l):
        r0 = pl.multiple_of(r * R, R)
        ot = ot_s[:, pl.ds(r0, R)].astype(BF)
        x = xs[pl.ds(r0, R), :] + lax.dot_general(ot, wo_ref[...], TN, preferred_element_type=F32)
        xn = _ln(x).astype(BF)
        h = lax.dot_general(xn, w1_ref[...], NT, preferred_element_type=F32) + b1_hbm[...].astype(F32).reshape(1, F)
        h = _gelu(h).astype(BF)
        x = x + jnp.dot(h, w2_ref[...], preferred_element_type=F32) + b2_hbm[...].astype(F32).reshape(1, D)
        xs[pl.ds(r0, R), :] = x
        o_ref[pl.ds(r0, R), :] = x.astype(BF)
        return l

    def ffn_it(i, l):
        @pl.when(jnp.logical_and(l == 1, i > 0))
        def _():
            for t in range(GF):
                o_cp((i - 1) * GF + t).start()
        for t in range(GF):
            ffn_blk(i * GF + t, l)
        return l

    def layer(l, _):
        @pl.when(l == 0)
        def _():
            x_in(0)
            x_in(1)
        xn_s[0:R, :] = _ln(xs[0:R, :]).astype(BF)
        for r in range(NB):
            if r == 1:
                @pl.when(l == 0)
                def _():
                    for rr in range(2, NB):
                        x_in(rr)
            if r + 1 < NB:
                xn_s[(r + 1) * R:(r + 2) * R, :] = _ln(xs[(r + 1) * R:(r + 2) * R, :]).astype(BF)
            v_blk(r)

        @pl.when(l == 0)
        def _():
            wq_cp[1].wait()
            wq_cp[2].wait()
        def qk_it(i, _):
            qk_blk(2 * i, 0)
            qk_blk(2 * i + 1, 0)
            return 0
        lax.fori_loop(0, NB // 2, qk_it, 0)

        @pl.when(l == 0)
        def _():
            for c in w_cp:
                c.start()
        attention()

        @pl.when(l == 0)
        def _():
            for c in w_cp:
                c.wait()
        lax.fori_loop(0, NB // GF, ffn_it, l)
        return 0

    wq_cp[0].wait()
    for r in range(1, NB):
        x_cp(r).start()
    wq_cp[1].start()
    wq_cp[2].start()
    lax.fori_loop(0, 2, layer, 0)
    for r in range(NB - GF, NB):
        o_cp(r).start()
    for r in range(NB):
        o_cp(r).wait()


@jax.jit
def pallas_interleave_layers__sliding_block__dense_activation_gelu__prompt_kernel(A_x, A_wqkv, A_wo, B_x, B_w1, B_b1, B_w2, B_b2):
    out = pl.pallas_call(
        _kernel,
        out_shape=jax.ShapeDtypeStruct((S, D), BF),
        in_specs=[pl.BlockSpec(memory_space=m) for m in (pl.ANY,) * 4 + (pltpu.VMEM, pl.ANY, pltpu.VMEM)],
        out_specs=pl.BlockSpec(memory_space=pl.ANY),
        scratch_shapes=[
            pltpu.VMEM((S, D), BF), pltpu.VMEM((D, 3 * D), BF), pltpu.VMEM((D, D), BF), pltpu.VMEM((F, D), BF),
            pltpu.VMEM((F, D), BF), pltpu.VMEM((S, D), BF),
            pltpu.SemaphoreType.DMA((2 * (S // R) + 7,)),
            pltpu.VMEM((S, D), F32), pltpu.VMEM((S, D), BF),
            pltpu.VMEM((8, S // 128, KC, 128), BF),
            pltpu.VMEM((8, S + W, 128), BF),
            pltpu.VMEM((H, (S + W) // 128, 32, 128), BF),
            pltpu.VMEM((D, S), F32),
            pltpu.VMEM((320, 512), F32),
            pltpu.VMEM((320, 512), F32),
            pltpu.VMEM((320, 512), F32),
            pltpu.VMEM((320, 512), F32),
            pltpu.VMEM((4, 320, 128), BF),
            pltpu.VMEM((4, 320, 128), BF),
            pltpu.VMEM((4, 320, 128), BF),
            pltpu.VMEM((4, 320, 128), BF),
        ],
        compiler_params=pltpu.CompilerParams(vmem_limit_bytes=100 * 1024 * 1024, flags={'XLA_TPU_EVENLY_DISTRIBUTE_CRITICAL_NODES': True}),
    )(A_x.reshape(S, D), A_wqkv, A_wo, B_w1.T, B_b1, B_w2, B_b2)
    return out.reshape(1, S, D)
```
